```python
import jax
import jax.numpy as jnp

def _softmax(x, axis=-1):
    return jax.nn.softmax(x, axis=axis)

def _gelu(x):
    return jax.nn.gelu(x, approximate=True)

def _silu(x):
    return jax.nn.silu(x)

def _sigmoid(x):
    return jax.nn.sigmoid(x)

def _layernorm(x, axis=-1, eps=1e-05):
    m = jnp.mean(x, axis=axis, keepdims=True)
    v = jnp.var(x, axis=axis, keepdims=True)
    return (x - m) / jnp.sqrt(v + eps)

def _scatter_add(tgt, idx, src, axis=0):
    return tgt.at[idx].add(src)

def _segment_sum(src, seg, n):
    return jax.ops.segment_sum(src, seg, n)

class _Rng:

    def __init__(self, key):
        self._k = key

    def _next(self):
        self._k, sub = jax.random.split(self._k)
        return sub

    def normal(self, shape):
        return jax.random.normal(self._next(), shape, dtype=jnp.bfloat16)

    def randint(self, lo, hi, shape):
        return jax.random.randint(self._next(), shape, lo, hi, dtype=jnp.int32)

    def uniform(self, shape, lo=0.0, hi=1.0):
        return jax.random.uniform(self._next(), shape, jnp.bfloat16, lo, hi)

    def permutation(self, n):
        return jax.random.permutation(self._next(), n)
kernel_name = 'standalone__dilated_atrous__vision'

def setup_inputs():
    _rng = _Rng(jax.random.key(int.from_bytes(__import__("os").urandom(4), "little")))
    _w = lambda a: (lambda t: t.astype(jnp.bfloat16) if jnp.issubdtype(t.dtype, jnp.floating) else t)(jnp.asarray(a))
    H = W = 384
    C = 384
    k = 1
    return {'x': _w((lambda *s: _rng.normal(s) * 0.05)(1, H, W, C)), 'w': _w((lambda *s: _rng.normal(s) * 0.05)(k, k, C, C) * (1.0 / (k * C ** 0.5)))}

def reference(x, w):
    B, H, W, C = x.shape
    k = 1
    rate = 2
    pad = (k - 1) * rate // 2
    xp = jnp.pad(x, ((0, 0), (pad, pad), (pad, pad), (0, 0)))
    out = jnp.zeros_like(x)
    for i in range(k):
        for j in range(k):
            tap = xp[:, i * rate:i * rate + H, j * rate:j * rate + W, :].copy()
            out = out + jnp.einsum('bhwc,co->bhwo', tap, w[i, j])
    return out
```

```python
import jax
import jax.numpy as jnp
import jax.experimental.pallas as pl
import jax.experimental.pallas.tpu as pltpu

_NREG = 8
_RS = 512
_SEG = 48
_GSW = 22
_BURST = 16
_K = 18


@jax.jit
def pallas_standalone__dilated_atrous__vision_kernel(
    x: jax.Array,
    w: jax.Array,
):
    B, H, W, C = x.shape
    Co = w.shape[-1]
    assert w.shape[:2] == (1, 1) and Co == C
    M = B * H * W
    nreg, rs, seg = _NREG, _RS, _SEG
    per = M // nreg
    assert per * nreg == M and per % rs == 0 and per % seg == 0
    G = per // rs
    NW = per // seg
    g_sw, burst, K = _GSW, _BURST, _K
    n2 = G - g_sw
    assert burst * seg <= g_sw * rs
    for t in range(n2):
        assert (burst + (t + 1) * K) * seg <= (g_sw + t + 1) * rs
    assert burst + n2 * K <= NW

    def kernel(x_hbm, w_ref, o_hbm, buf, rsem, osem):
        def rd(j):
            rows = pl.ds(j * rs, rs)
            return pltpu.make_async_copy(x_hbm.at[:, rows], buf.at[:, rows], rsem.at[j])

        def issue_writes(lo, n):
            def body(i, c):
                rows = pl.ds(pl.multiple_of((lo + i) * seg, 16), seg)
                pltpu.make_async_copy(buf.at[:, rows], o_hbm.at[:, rows], osem).start()
                return c
            jax.lax.fori_loop(0, n, body, 0)

        def compute(g):
            rows = pl.ds(pl.multiple_of(g * rs, rs), rs)
            xv = buf[:, rows, :].reshape(nreg * rs, C)
            y = jnp.dot(xv, w_ref[...], preferred_element_type=jnp.float32)
            buf[:, rows, :] = y.astype(buf.dtype).reshape(nreg, rs, Co)

        for j in range(G):
            rd(j).start()

        def phase1(j, c):
            rd(j).wait()
            compute(j)
            return c
        jax.lax.fori_loop(0, g_sw, phase1, 0)

        for j in range(g_sw, G):
            rd(j).wait()
        issue_writes(0, burst)

        def phase2(t, c):
            compute(g_sw + t)
            issue_writes(burst + t * K, K)
            return c
        jax.lax.fori_loop(0, n2, phase2, 0)

        issue_writes(burst + n2 * K, NW - burst - n2 * K)
        pltpu.make_async_copy(buf, o_hbm, osem).wait()

    out = pl.pallas_call(
        kernel,
        in_specs=[
            pl.BlockSpec(memory_space=pl.ANY),
            pl.BlockSpec(memory_space=pltpu.VMEM),
        ],
        out_specs=pl.BlockSpec(memory_space=pl.ANY),
        out_shape=jax.ShapeDtypeStruct((nreg, per, Co), x.dtype),
        scratch_shapes=[
            pltpu.VMEM((nreg, per, C), x.dtype),
            pltpu.SemaphoreType.DMA((G,)),
            pltpu.SemaphoreType.DMA(()),
        ],
        compiler_params=pltpu.CompilerParams(vmem_limit_bytes=124 * 1024 * 1024),
    )(x.reshape(nreg, per, C), w.reshape(C, Co))
    return out.reshape(B, H, W, Co)
```

```python
import jax
import jax.numpy as jnp
from jax import lax
import jax.experimental.pallas as pl
import jax.experimental.pallas.tpu as pltpu

_NREG = 6
_S = 2048
_RSEG = 32
_WSEG = 16
_RS = 256
_P0 = 32
_KR = 16
_TAIL = 6
_W0 = 60
_KW = 27
_UNROLL = 4


@jax.jit
def pallas_standalone__dilated_atrous__vision_kernel(
    x: jax.Array,
    w: jax.Array,
):
    B, H, W, C = x.shape
    Co = w.shape[-1]
    assert w.shape == (1, 1, C, Co) and Co == C
    M = B * H * W
    nreg, S, rseg, wseg, rs = _NREG, _S, _RSEG, _WSEG, _RS
    P0, kr, tail, W0, kw = _P0, _KR, _TAIL, _W0, _KW
    nsuper = M // (nreg * S)
    assert nsuper * nreg * S == M
    lg = S.bit_length() - 1
    assert S == 1 << lg
    h = nreg // 2
    L = nsuper * S
    assert S % rs == 0 and rs % rseg == 0 and S % wseg == 0
    assert rseg % 16 == 0 and wseg % 16 == 0
    NP, NW, G = L // rseg, L // wseg, L // rs
    ppc = rs // rseg
    lgp = ppc.bit_length() - 1
    assert ppc == 1 << lgp
    cps = S // rs
    g_sw = (NP - tail - P0) // kr
    assert kr >= ppc
    n2 = G - g_sw
    assert W0 * wseg <= g_sw * rs and W0 + n2 * kw <= NW
    for t in range(n2):
        assert (W0 + (t + 1) * kw) * wseg <= (g_sw + t + 1) * rs
    s_al = -(-g_sw // cps)
    g_al = s_al * cps
    off = g_al - s_al
    TAIL = g_al + (nsuper - s_al)
    assert 0 < tail * rseg < S and s_al < nsuper

    def kernel(x_hbm, w_hbm, o_hbm, buf, wbuf, osem):
        def pos(v, n, align=16):
            if isinstance(v, int):
                return v >> lg, pl.ds(v & (S - 1), n)
            return (lax.shift_right_logical(v, lg),
                    pl.ds(pl.multiple_of(v & (S - 1), align), n))

        def loop(lo, hi, fn, u=1):
            n = hi - lo

            def body(t, c):
                for k in range(u):
                    fn(lo + t * u + k)
                return c
            if n // u > 0:
                lax.fori_loop(0, n // u, body, 0)
            for k in range(lo + n // u * u, hi):
                fn(k)

        def compute(g):
            s, rows = pos(g * rs, rs, rs)
            xv = buf[s, :, rows, :].reshape(nreg * rs, C)
            y = jnp.dot(xv, wbuf[...], preferred_element_type=jnp.float32)
            buf[s, :, rows, :] = y.astype(buf.dtype).reshape(nreg, rs, Co)

        def write_one(i):
            s, rows = pos(i * wseg, wseg)
            pltpu.make_async_copy(buf.at[s, :, rows], o_hbm.at[s, :, rows], osem).start()

        def read_phase(rsem, wsem):
            def read_pair(p, semi=None):
                s, rows = pos(p * rseg, rseg)
                if semi is None:
                    if isinstance(p, int):
                        semi = min(p >> lgp, off + s)
                    else:
                        semi = jnp.minimum(lax.shift_right_logical(p, lgp), off + s)
                sem = rsem.at[semi]
                pltpu.make_async_copy(
                    x_hbm.at[s, 0:h, rows], buf.at[s, 0:h, rows], sem).start(priority=0)
                pltpu.make_async_copy(
                    x_hbm.at[s, h:nreg, rows], buf.at[s, h:nreg, rows], sem).start(priority=1)

            def wait_region(s, rows, semi):
                pltpu.make_async_copy(
                    x_hbm.at[s, :, rows], buf.at[s, :, rows], rsem.at[semi]).wait()

            wcp = pltpu.make_async_copy(w_hbm, wbuf, wsem)
            wcp.start()
            loop(0, P0, read_pair, _UNROLL)
            wcp.wait()

            def step(t):
                for k in range(kr):
                    read_pair(P0 + t * kr + k)
                wait_region(*pos(t * rs, rs, rs), t)
                compute(t)
            loop(0, g_sw, step)

            loop(P0 + g_sw * kr, NP - tail, read_pair, _UNROLL)
            for p in range(NP - tail, NP):
                read_pair(p, TAIL)
            for g in range(g_sw, g_al):
                wait_region(*pos(g * rs, rs), g)
            for s in range(s_al, nsuper):
                n = S - (tail * rseg if s == nsuper - 1 else 0)
                wait_region(s, pl.ds(0, n), off + s)
            loop(0, W0, write_one, _UNROLL)
            wait_region(nsuper - 1, pl.ds(S - tail * rseg, tail * rseg), TAIL)

        pl.run_scoped(
            read_phase,
            pltpu.SemaphoreType.DMA((TAIL + 1,)),
            pltpu.SemaphoreType.DMA(()),
        )

        def step2(t):
            compute(g_sw + t)
            for k in range(kw):
                write_one(W0 + t * kw + k)
        loop(0, n2, step2)

        loop(W0 + n2 * kw, NW, write_one, _UNROLL)
        pltpu.make_async_copy(buf, o_hbm, osem).wait()

    out = pl.pallas_call(
        kernel,
        in_specs=[
            pl.BlockSpec(memory_space=pl.ANY),
            pl.BlockSpec(memory_space=pl.ANY),
        ],
        out_specs=pl.BlockSpec(memory_space=pl.ANY),
        out_shape=jax.ShapeDtypeStruct((nsuper, nreg, S, Co), x.dtype),
        scratch_shapes=[
            pltpu.VMEM((nsuper, nreg, S, C), x.dtype),
            pltpu.VMEM((C, Co), w.dtype),
            pltpu.SemaphoreType.DMA(()),
        ],
        compiler_params=pltpu.CompilerParams(
            vmem_limit_bytes=124 * 1024 * 1024,
            disable_bounds_checks=True,
        ),
    )(x.reshape(nsuper, nreg, S, C), w.reshape(C, Co))
    return out.reshape(B, H, W, Co)
```

```python
import jax
import jax.numpy as jnp
from jax import lax
import jax.experimental.pallas as pl
import jax.experimental.pallas.tpu as pltpu

_CFG = dict(
    S=2048,
    RG=12,
    WG=6,
    rseg=8,
    wseg=16,
    rs1=128,
    rs2=256,
    n1=3,
    kr=31,
    tail=12,
    w0=60,
    kw=27,
)
_UNROLL = 4


def _matmul_rows(x2, w2, *, S, RG, WG, rseg, wseg, rs1, rs2, n1, kr, tail, w0, kw,
                 interpret=False):
    M, C = x2.shape
    Co = w2.shape[1]
    assert Co == C
    NB = M // S
    lg = S.bit_length() - 1
    assert S == 1 << lg and NB * S == M and NB % RG == 0 and NB % WG == 0
    assert S % rs1 == 0 and S % rs2 == 0 and rs1 % rseg == 0 and S % wseg == 0
    assert rs1 % 16 == 0 and rs2 % 16 == 0 and rseg % 8 == 0 and wseg % 8 == 0
    h = RG // 2
    NRG, NWG = NB // RG, NB // WG
    NP = NRG * S // rseg
    NW = NWG * S // wseg
    ppc = rs1 // rseg
    lgp = ppc.bit_length() - 1
    assert ppc == 1 << lgp
    G1 = n1 * (S // rs1)
    p0 = NP - tail - G1 * kr
    assert p0 >= 0 and kr >= ppc
    assert (n1 * RG) % WG == 0 and n1 < NRG and 0 < tail * rseg < S
    v2 = n1 * RG // WG * S
    n2 = (NWG * S - v2) // rs2
    assert w0 * wseg <= v2 and w0 + n2 * kw <= NW
    for t in range(n2):
        assert (w0 + (t + 1) * kw) * wseg <= v2 + (t + 1) * rs2
    off = G1 - n1
    TAIL = G1 + NRG - n1

    def kernel(x_hbm, w_hbm, o_hbm, buf, wbuf, osem):
        def pos(v, n):
            if isinstance(v, int):
                return v >> lg, pl.ds(v & (S - 1), n)
            return (lax.shift_right_logical(v, lg),
                    pl.ds(pl.multiple_of(v & (S - 1), n & -n), n))

        def loop(lo, hi, fn, u=1):
            n = hi - lo

            def body(t, c):
                for k in range(u):
                    fn(lo + t * u + k)
                return c
            if n // u > 0:
                lax.fori_loop(0, n // u, body, 0)
            for k in range(lo + n // u * u, hi):
                fn(k)

        def compute(v, grp, rs):
            s, rows = pos(v, rs)
            blks = pl.ds(s * grp, grp)
            xv = buf[blks, rows, :].reshape(grp * rs, C)
            y = jnp.dot(xv, wbuf[...], preferred_element_type=jnp.float32)
            buf[blks, rows, :] = y.astype(buf.dtype).reshape(grp, rs, Co)

        def write_one(i):
            s, rows = pos(i * wseg, wseg)
            blks = pl.ds(s * WG, WG)
            pltpu.make_async_copy(buf.at[blks, rows], o_hbm.at[blks, rows], osem).start()

        def read_phase(rsem, wsem):
            def read_pair(p, semi=None):
                s, rows = pos(p * rseg, rseg)
                if semi is None:
                    if isinstance(p, int):
                        semi = min(p >> lgp, off + s)
                    else:
                        semi = jnp.minimum(lax.shift_right_logical(p, lgp), off + s)
                sem = rsem.at[semi]
                a, b = pl.ds(s * RG, h), pl.ds(s * RG + h, RG - h)
                pltpu.make_async_copy(
                    x_hbm.at[a, rows], buf.at[a, rows], sem).start(priority=0)
                pltpu.make_async_copy(
                    x_hbm.at[b, rows], buf.at[b, rows], sem).start(priority=1)

            def wait_region(s, rows, semi):
                blks = pl.ds(s * RG, RG)
                pltpu.make_async_copy(
                    x_hbm.at[blks, rows], buf.at[blks, rows], rsem.at[semi]).wait()

            wcp = pltpu.make_async_copy(w_hbm, wbuf, wsem)
            wcp.start()
            loop(0, p0, read_pair, _UNROLL)
            wcp.wait()

            def step(t):
                for k in range(kr):
                    read_pair(p0 + t * kr + k)
                wait_region(*pos(t * rs1, rs1), t)
                compute(t * rs1, RG, rs1)
            loop(0, G1, step)

            for p in range(NP - tail, NP):
                read_pair(p, TAIL)
            for s in range(n1, NRG):
                n = S - (tail * rseg if s == NRG - 1 else 0)
                wait_region(s, pl.ds(0, n), off + s)
            loop(0, w0, write_one, _UNROLL)
            wait_region(NRG - 1, pl.ds(S - tail * rseg, tail * rseg), TAIL)

        pl.run_scoped(
            read_phase,
            pltpu.SemaphoreType.DMA((TAIL + 1,)),
            pltpu.SemaphoreType.DMA(()),
        )

        def step2(t):
            compute(v2 + t * rs2, WG, rs2)
            for k in range(kw):
                write_one(w0 + t * kw + k)
        loop(0, n2, step2)

        loop(w0 + n2 * kw, NW, write_one, _UNROLL)
        pltpu.make_async_copy(buf, o_hbm, osem).wait()

    return pl.pallas_call(
        kernel,
        in_specs=[
            pl.BlockSpec(memory_space=pl.ANY),
            pl.BlockSpec(memory_space=pl.ANY),
        ],
        out_specs=pl.BlockSpec(memory_space=pl.ANY),
        out_shape=jax.ShapeDtypeStruct((NB, S, Co), x2.dtype),
        scratch_shapes=[
            pltpu.VMEM((NB, S, C), x2.dtype),
            pltpu.VMEM((C, Co), w2.dtype),
            pltpu.SemaphoreType.DMA(()),
        ],
        compiler_params=pltpu.CompilerParams(
            vmem_limit_bytes=124 * 1024 * 1024,
            disable_bounds_checks=True,
        ),
        interpret=interpret,
    )(x2.reshape(NB, S, C), w2)


@jax.jit
def pallas_standalone__dilated_atrous__vision_kernel(
    x: jax.Array,
    w: jax.Array,
):
    B, H, W, C = x.shape
    Co = w.shape[-1]
    assert w.shape == (1, 1, C, Co)
    out = _matmul_rows(x.reshape(B * H * W, C), w.reshape(C, Co), **_CFG)
    return out.reshape(B, H, W, Co)
```
